```python
import os as _os
_os.environ.setdefault("JAX_PLATFORMS", "cpu")
import jax
import jax.numpy as jnp

def _softmax(x, axis=-1):
    return jax.nn.softmax(x, axis=axis)
def _gelu(x):
    return jax.nn.gelu(x, approximate=True)
def _silu(x):
    return jax.nn.silu(x)
def _sigmoid(x):
    return jax.nn.sigmoid(x)
def _layernorm(x, axis=-1, eps=1e-5):
    m = jnp.mean(x, axis=axis, keepdims=True)
    v = jnp.var(x, axis=axis, keepdims=True)
    return (x - m) / jnp.sqrt(v + eps)
def _scatter_add(tgt, idx, src, axis=0):
    return tgt.at[idx].add(src)
def _segment_sum(src, seg, n):
    return jax.ops.segment_sum(src, seg, n)
class _Rng:
    def __init__(self, key):
        self._k = key
    def _next(self):
        self._k, sub = jax.random.split(self._k)
        return sub
    def normal(self, shape):
        return jax.random.normal(self._next(), shape, dtype=jnp.bfloat16)
    def randint(self, lo, hi, shape):
        return jax.random.randint(self._next(), shape, lo, hi, dtype=jnp.int32)
    def uniform(self, shape, lo=0.0, hi=1.0):
        return jax.random.uniform(self._next(), shape, jnp.bfloat16, lo, hi)
    def permutation(self, n):
        return jax.random.permutation(self._next(), n)


kernel_name = 'standalone__mha_block_cached__near_ridge'

def setup_inputs():
    _rng = _Rng(jax.random.key(int.from_bytes(__import__("os").urandom(4), "little")))
    _w = (lambda a: (lambda t: t.astype(jnp.bfloat16) if jnp.issubdtype(t.dtype, jnp.floating) else t)(jnp.asarray(a)))
    B, Sq, D = 8, 96, 576
    H, Sk, Dh = 32, 96, 128
    return {
        "x": _w((lambda *s: _rng.normal(s) * 0.8)(B, Sq, D)),
        "k_cache": _w((lambda *s: _rng.normal(s) * 0.8)(B, H, Sk, Dh)),
        "v_cache": _w((lambda *s: _rng.normal(s) * 0.05)(B, H, Sk, Dh)),
        "wq": _w((lambda *s: _rng.normal(s) * 0.8)(D, H * Dh) * (D ** -0.5)),
        "wo": _w((lambda *s: _rng.normal(s) * 0.05)(H * Dh, D) * ((H * Dh) ** -0.5)),
    }

def reference(x, k_cache, v_cache, wq, wo):
    B, Sq, D = x.shape
    H, Dh = 32, 128
    q = (lambda x, *d: x.transpose(*d))((x @ wq).reshape(B, Sq, H, Dh), 0, 2, 1, 3)
    scores = jnp.einsum("bhqd,bhkd->bhqk", q, k_cache) * (Dh ** -0.5)
    p = _softmax(scores, axis=-1)
    o = jnp.einsum("bhqk,bhkd->bhqd", p, v_cache)
    return (lambda x, *d: x.transpose(*d))(o, 0, 2, 1, 3).reshape(B, Sq, H * Dh) @ wo
```

```python
import functools
import jax
import jax.numpy as jnp
from jax import lax
import jax.experimental.pallas as pl
import jax.experimental.pallas.tpu as pltpu

G = 4

@jax.jit
def pallas_standalone__mha_block_cached__near_ridge_kernel(x, k_cache, v_cache, wq, wo):
    B, Sq, D = x.shape
    _, H, Sk, Dh = k_cache.shape
    M = B * Sq
    scale = Dh ** -0.5
    x2 = x.reshape(M, D)
    woT = wo.T
    nsteps = H // G

    def kernel(x_ref, wq_ref, k_ref, v_ref, wo_ref, o_ref, acc_ref, q_ref, a_ref):
        g = pl.program_id(0)
        q = jnp.dot(x_ref[...], wq_ref[...], preferred_element_type=jnp.float32)
        q_ref[...] = (q * scale).astype(jnp.bfloat16)
        for b in range(B):
            for h in range(G):
                qb = q_ref[b * Sq:(b + 1) * Sq, h * Dh:(h + 1) * Dh]
                s = lax.dot_general(qb, k_ref[b, h], (((1,), (1,)), ((), ())),
                                    preferred_element_type=jnp.float32)
                m = jnp.max(s, axis=-1, keepdims=True)
                p = jnp.exp(s - m)
                l = jnp.sum(p, axis=-1, keepdims=True)
                o = jnp.dot(p.astype(jnp.bfloat16), v_ref[b, h], preferred_element_type=jnp.float32)
                o = o * (1.0 / l)
                a_ref[b * Sq:(b + 1) * Sq, h * Dh:(h + 1) * Dh] = o.astype(jnp.bfloat16)
        contrib = lax.dot_general(a_ref[...], wo_ref[...], (((1,), (1,)), ((), ())), preferred_element_type=jnp.float32)

        @pl.when(g == 0)
        def _():
            acc_ref[...] = contrib

        @pl.when(g > 0)
        def _():
            acc_ref[...] += contrib

        @pl.when(g == nsteps - 1)
        def _():
            o_ref[...] = acc_ref[...].astype(o_ref.dtype)

    out = pl.pallas_call(
        kernel,
        grid=(nsteps,),
        in_specs=[
            pl.BlockSpec((M, D), lambda g: (0, 0)),
            pl.BlockSpec((D, G * Dh), lambda g: (0, g)),
            pl.BlockSpec((B, G, Sk, Dh), lambda g: (0, g, 0, 0)),
            pl.BlockSpec((B, G, Sk, Dh), lambda g: (0, g, 0, 0)),
            pl.BlockSpec((D, G * Dh), lambda g: (0, g)),
        ],
        out_specs=pl.BlockSpec((M, D), lambda g: (0, 0)),
        out_shape=jax.ShapeDtypeStruct((M, D), x.dtype),
        scratch_shapes=[
            pltpu.VMEM((M, D), jnp.float32),
            pltpu.VMEM((M, G * Dh), jnp.bfloat16),
            pltpu.VMEM((M, G * Dh), jnp.bfloat16),
        ],
        compiler_params=pltpu.CompilerParams(
            dimension_semantics=("arbitrary",),
            vmem_limit_bytes=100 * 1024 * 1024,
        ),
    )(x2, wq, k_cache, v_cache, woT)
    return out.reshape(B, Sq, D)
```

```python
import jax
import jax.numpy as jnp
from jax import lax
import jax.experimental.pallas as pl
import jax.experimental.pallas.tpu as pltpu

G = 2
OM = 288
NPS = 4
NAT = (3, 4, 5)
CSPLIT = ((0, 256), (256, 512), (512, 576))

_NT = (((1,), (1,)), ((), ()))


@jax.jit
def pallas_standalone__mha_block_cached__near_ridge_kernel(x, k_cache, v_cache, wq, wo):
    B, Sq, D = x.shape
    _, H, Sk, Dh = k_cache.shape
    M = B * Sq
    scale = Dh ** -0.5
    x2 = x.reshape(M, D)
    woT = wo.T
    n = H // G
    NP = n // 2
    GD = G * Dh
    XR = 2 * Sq
    NB = NP - 4
    NT = M // 128
    SEM_A = 5
    SEM_E = 4
    SEM_OUT = SEM_A
    NSEM = 6

    def kernel(x_hbm, wq_hbm, k_hbm, v_hbm, wo_hbm, o_hbm,
               x_v, wq_v, k_v, v_v, wo_v, acc_ref, q_v, p_v, a_v, o_v, acct_v, sems):
        def half(s):
            return slice(s * GD, (s + 1) * GD)

        def cp_x(c, s):
            sl = pl.ds(c * XR, XR)
            return pltpu.make_async_copy(x_hbm.at[sl], x_v.at[sl], sems.at[s])

        def cp_w_pair(w_hbm, w_v, pr, s):
            c0 = pr * 2 * GD
            if not isinstance(c0, int):
                c0 = pl.multiple_of(c0, 2 * GD)
            return pltpu.make_async_copy(w_hbm.at[:, pl.ds(c0, 2 * GD)], w_v.at[pr], sems.at[s])

        def cp_w_unit(w_hbm, w_v, pr, hf, s):
            c0 = (pr * 2 + hf) * GD
            return pltpu.make_async_copy(w_hbm.at[:, pl.ds(c0, GD)], w_v.at[pr, :, half(hf)],
                                         sems.at[s])

        def cp_kv(c_hbm, c_v, u, nu, s):
            hs = pl.ds(u * G, nu * G)
            return pltpu.make_async_copy(c_hbm.at[:, hs], c_v.at[:, hs], sems.at[s])

        def cp_out(t):
            sl = pl.ds(t * 128, 128)
            return pltpu.make_async_copy(o_v.at[sl], o_hbm.at[sl], sems.at[SEM_OUT])

        def cp_last(c0, c1):
            sl = pl.ds((NT - 1) * 128, 128)
            cl = pl.ds(c0, c1 - c0)
            return pltpu.make_async_copy(o_v.at[sl, cl], o_hbm.at[sl, cl], sems.at[SEM_OUT])

        def set_a():
            s = SEM_A
            return [cp_kv(k_hbm, k_v, 0, 2, s), cp_w_pair(wq_hbm, wq_v, 2, s),
                    cp_kv(v_hbm, v_v, 0, 2, s)]

        def set_b(pr, s):
            return [cp_kv(k_hbm, k_v, 2 * pr, 2, s), cp_w_pair(wo_hbm, wo_v, pr - 1, s),
                    cp_w_pair(wq_hbm, wq_v, pr + 2, s), cp_kv(v_hbm, v_v, 2 * pr, 2, s)]

        def set_e():
            s = SEM_E
            return set_b(NP - 3, s) + [
                cp_kv(k_hbm, k_v, n - 4, 4, s), cp_w_pair(wo_hbm, wo_v, NP - 3, s),
                cp_kv(v_hbm, v_v, n - 4, 4, s), cp_w_pair(wo_hbm, wo_v, NP - 2, s),
                cp_w_pair(wo_hbm, wo_v, NP - 1, s)]

        pro_sets = [
            [cp_w_unit(wq_hbm, wq_v, 0, 0, 0), cp_x(0, 0)],
            [cp_x(1, 1)],
            [cp_w_unit(wq_hbm, wq_v, 0, 1, 2)],
            [cp_x(2, 3), cp_x(3, 3)],
            [cp_w_pair(wq_hbm, wq_v, 1, 4)],
        ]

        def start(cps):
            for cp in cps:
                cp.start()

        def wait(cps):
            for cp in cps:
                cp.wait()

        for st in pro_sets:
            start(st)
        start(set_a())

        acc_ref[...] = jnp.zeros_like(acc_ref)

        def qp(pr, hf, qs, b):
            r0, r1 = b * Sq, (b + 1) * Sq
            q = jnp.dot(x_v[r0:r1, :], wq_v[pr, :, half(hf)], preferred_element_type=jnp.float32)
            q_v[qs, r0:r1, :] = (q * scale).astype(jnp.bfloat16)

        def qk(u, qs, b, ps=0):
            for h in range(G):
                qb = q_v[qs, b * Sq:(b + 1) * Sq, h * Dh:(h + 1) * Dh]
                s = lax.dot_general(qb, k_v[b, u * G + h], _NT, preferred_element_type=jnp.float32)
                m = jnp.max(s, axis=-1, keepdims=True)
                p = jnp.exp(s - m)
                l = jnp.sum(p, axis=-1, keepdims=True)
                p_v[b % NPS, ps * G + h] = (p * pl.reciprocal(l, approx=True)).astype(jnp.bfloat16)

        def pv(u, slot, b, ps=0):
            for h in range(G):
                o = jnp.dot(p_v[b % NPS, ps * G + h], v_v[b, u * G + h],
                            preferred_element_type=jnp.float32)
                c0 = slot * GD + h * Dh
                a_v[b * Sq:(b + 1) * Sq, c0:c0 + Dh] = o.astype(jnp.bfloat16)

        def op(pr, slot, t):
            cs = slice(t * 128, (t + 1) * 128)
            at = a_v[cs, half(slot)]
            for r0 in range(0, D, OM):
                c = lax.dot_general(wo_v[pr, r0:r0 + OM, half(slot)], at, _NT,
                                    preferred_element_type=jnp.float32)
                acc_ref[r0:r0 + OM, cs] += c

        def op_nat(t, c0=0, c1=D):
            cs = slice(t * 128, (t + 1) * 128)
            tot = acct_v[NAT.index(t), :, c0:c1] + lax.dot_general(
                a_v[cs, :], wo_v[NP - 1, c0:c1, :], _NT, preferred_element_type=jnp.float32)
            o_v[cs, c0:c1] = tot.astype(o_v.dtype)

        def op2(pr, t):
            cs = slice(t * 128, (t + 1) * 128)
            if pr == NP - 1 and t in NAT:
                op_nat(t)
                return
            tot = acc_ref[:, cs] + lax.dot_general(wo_v[pr], a_v[cs, :], _NT,
                                                   preferred_element_type=jnp.float32)
            if pr == NP - 2 and t in NAT:
                acct_v[NAT.index(t)] = tot.T
            elif pr < NP - 1:
                acc_ref[:, cs] = tot
            else:
                o_v[cs, :] = tot.T.astype(o_v.dtype)

        def tail_pv(u, slot):
            pv(u, slot, B - 2)
            pv(u, slot, B - 1)

        OT = {0: 1, 1: 2, 3: 3, 4: 4, 5: 5}

        def unit_a(u):
            if u > 0:
                tail_pv(u - 1, u - 1)
            qk(u, u, 0)
            qk(u, u, 1)
            qp(2, u, u, 0)
            qk(u, u, 2)
            qp(2, u, u, 1)
            for b in range(B - 3):
                pv(u, u, b)
                qk(u, u, b + 3)
                qp(2, u, u, b + 2)
            pv(u, u, B - 3)
            qp(2, u, u, B - 1)

        def unit_b(pr, hf, qs):
            u = 2 * pr + hf
            tail_pv(u - 1, 1 - hf)
            qk(u, qs, 0)
            qk(u, qs, 1)
            op(pr - 1, hf, 0)
            qp(pr + 2, hf, qs, 0)
            for b in range(B - 2):
                pv(u, hf, b)
                qk(u, qs, b + 2)
                if b in OT:
                    op(pr - 1, hf, OT[b])
                qp(pr + 2, hf, qs, b + 1)
            qp(pr + 2, hf, qs, B - 1)

        def pair_b(pr):
            qb = (pr % 2) * 2
            unit_b(pr, 0, qb)
            unit_b(pr, 1, qb + 1)

        def qk2(pr, b):
            qb = (pr % 2) * 2
            qk(2 * pr, qb, b, 0)
            qk(2 * pr + 1, qb + 1, b, 1)

        def pv2(pr, b):
            pv(2 * pr, 0, b, 0)
            pv(2 * pr + 1, 1, b, 1)

        for c, st in enumerate(pro_sets):
            wait(st)
            start(set_b(c + 1, c) if c < NB else set_e())
            if c < 2:
                qp(0, 0, 0, 2 * c)
                qp(0, 0, 0, 2 * c + 1)
            elif c == 2:
                for b in range(4):
                    qp(0, 1, 1, b)
            elif c == 3:
                for b in range(4, B):
                    qp(0, 0, 0, b)
                    qp(0, 1, 1, b)
            else:
                for b in range(B):
                    qp(1, 0, 2, b)
                    qp(1, 1, 3, b)

        wait(set_a())
        unit_a(0)
        unit_a(1)

        def body_b(pr, carry):
            wait(set_b(pr, pr - 1))
            pair_b(pr)
            return carry

        lax.fori_loop(1, NB + 1, body_b, 0)

        wait(set_e())
        pair_b(NP - 3)
        c, e = NP - 2, NP - 1
        tail_pv(2 * c - 1, 1)
        qk2(c, 0); qk2(c, 1); op2(c - 1, 0)
        pv2(c, 0); qk2(c, 2); op2(c - 1, 1)
        pv2(c, 1); qk2(c, 3); op2(c - 1, 2)
        pv2(c, 2); qk2(c, 4); op2(c - 1, 3)
        pv2(c, 3); qk2(c, 5); op2(c - 1, 4)
        pv2(c, 4); qk2(c, 6); qk2(c, 7); op2(c - 1, 5)
        pv2(c, 5); qk2(e, 0); op2(c, 0)
        pv2(c, 6); pv2(c, 7); qk2(e, 1); op2(c, 1)
        pv2(e, 0); qk2(e, 2); op2(c, 2)
        pv2(e, 1); qk2(e, 3); op2(c, 3)
        pv2(e, 2); qk2(e, 4); op2(c, 4)
        pv2(e, 3); qk2(e, 5); op2(c, 5)
        pv2(e, 4); qk2(e, 6); op2(e, 0)
        cp_out(0).start()
        pv2(e, 5); qk2(e, 7); op2(e, 1)
        cp_out(1).start()
        op2(e, 2)
        cp_out(2).start()
        pv2(e, 6); op2(e, 3)
        cp_out(3).start()
        pv2(e, 7); op2(e, 4)
        cp_out(4).start()
        for (c0, c1) in CSPLIT:
            op_nat(NT - 1, c0, c1)
            cp_last(c0, c1).start()
        for t in range(NT - 1):
            cp_out(t).wait()
        for (c0, c1) in CSPLIT:
            cp_last(c0, c1).wait()

    out = pl.pallas_call(
        kernel,
        in_specs=[pl.BlockSpec(memory_space=pl.ANY)] * 5,
        out_specs=pl.BlockSpec(memory_space=pl.ANY),
        out_shape=jax.ShapeDtypeStruct((M, D), x.dtype),
        scratch_shapes=[
            pltpu.VMEM((M, D), jnp.bfloat16),
            pltpu.VMEM((NP, D, 2 * GD), jnp.bfloat16),
            pltpu.VMEM((B, H, Sk, Dh), jnp.bfloat16),
            pltpu.VMEM((B, H, Sk, Dh), jnp.bfloat16),
            pltpu.VMEM((NP, D, 2 * GD), jnp.bfloat16),
            pltpu.VMEM((D, M), jnp.float32),
            pltpu.VMEM((4, M, GD), jnp.bfloat16),
            pltpu.VMEM((NPS, 2 * G, Sq, Sk), jnp.bfloat16),
            pltpu.VMEM((M, 2 * GD), jnp.bfloat16),
            pltpu.VMEM((M, D), jnp.bfloat16),
            pltpu.VMEM((len(NAT), 128, D), jnp.float32),
            pltpu.SemaphoreType.DMA((NSEM,)),
        ],
        compiler_params=pltpu.CompilerParams(
            vmem_limit_bytes=100 * 1024 * 1024,
        ),
    )(x2, wq, k_cache, v_cache, woT)
    return out.reshape(B, Sq, D)
```

```python
import jax
import jax.numpy as jnp
from jax import lax
import jax.experimental.pallas as pl
import jax.experimental.pallas.tpu as pltpu

G = 2
OM = 288
NPS = 4
NAT = (3, 4, 5)
CSPLIT = ((0, 256), (256, 512), (512, 576))

_NT = (((1,), (1,)), ((), ()))
KSPLIT = ((512, 576), (0, 256), (256, 512))
PM = 192


@jax.jit
def pallas_standalone__mha_block_cached__near_ridge_kernel(x, k_cache, v_cache, wq, wo):
    B, Sq, D = x.shape
    _, H, Sk, Dh = k_cache.shape
    M = B * Sq
    scale = Dh ** -0.5
    x2 = x.reshape(M, D)
    woT = wo.T
    n = H // G
    NP = n // 2
    GD = G * Dh
    NB = NP - 4
    NT = M // 128
    NK = len(KSPLIT)
    KM = KSPLIT[0][0]
    REM = {0: (NP - 1,)}
    RSLOT = {}
    for blk in sorted(REM):
        for pr in REM[blk]:
            RSLOT[pr] = 2 + len(RSLOT)
    SEM_A = NB
    SEM_E = NB + 1
    SEM_OUT = SEM_A
    NSEM = NB + 2
    assert NK <= NB

    def kernel(x_hbm, wq_hbm, k_hbm, v_hbm, wo_hbm, o_hbm,
               x_v, wq_v, k_v, v_v, wo_v, acc_ref, q_v, p_v, a_v, o_v, acct_v, qacc_v, sems):
        def half(s):
            return slice(s * GD, (s + 1) * GD)

        def cp_w_pair(w_hbm, w_v, pr, s):
            c0 = pr * 2 * GD
            if not isinstance(c0, int):
                c0 = pl.multiple_of(c0, 2 * GD)
            elif w_v is wq_v and pr in RSLOT:
                km = pl.ds(0, KM)
                return pltpu.make_async_copy(w_hbm.at[km, pl.ds(c0, 2 * GD)], w_v.at[pr, km, :],
                                             sems.at[s])
            return pltpu.make_async_copy(w_hbm.at[:, pl.ds(c0, 2 * GD)], w_v.at[pr], sems.at[s])

        def cp_kv(c_hbm, c_v, u, nu, s):
            hs = pl.ds(u * G, nu * G)
            return pltpu.make_async_copy(c_hbm.at[:, hs], c_v.at[:, hs], sems.at[s])

        def cp_out(t):
            sl = pl.ds(t * 128, 128)
            return pltpu.make_async_copy(o_v.at[sl], o_hbm.at[sl], sems.at[SEM_OUT])

        def cp_last(c0, c1):
            sl = pl.ds((NT - 1) * 128, 128)
            cl = pl.ds(c0, c1 - c0)
            return pltpu.make_async_copy(o_v.at[sl, cl], o_hbm.at[sl, cl], sems.at[SEM_OUT])

        def set_a():
            s = SEM_A
            return [cp_kv(k_hbm, k_v, 0, 2, s), cp_w_pair(wq_hbm, wq_v, 2, s),
                    cp_kv(v_hbm, v_v, 0, 2, s)]

        def set_b(pr, s):
            return [cp_kv(k_hbm, k_v, 2 * pr, 2, s), cp_w_pair(wo_hbm, wo_v, pr - 1, s),
                    cp_w_pair(wq_hbm, wq_v, pr + 2, s), cp_kv(v_hbm, v_v, 2 * pr, 2, s)]

        def set_e():
            s = SEM_E
            return set_b(NP - 3, s) + [
                cp_kv(k_hbm, k_v, n - 4, 4, s), cp_w_pair(wo_hbm, wo_v, NP - 3, s),
                cp_kv(v_hbm, v_v, n - 4, 4, s), cp_w_pair(wo_hbm, wo_v, NP - 2, s),
                cp_w_pair(wo_hbm, wo_v, NP - 1, s)]

        def set_p(i):
            k0, k1 = KSPLIT[i]
            ks = pl.ds(k0, k1 - k0)
            r = [pltpu.make_async_copy(x_hbm.at[:, ks], x_v.at[:, ks], sems.at[i])]
            for pr in range(2):
                r.append(pltpu.make_async_copy(wq_hbm.at[ks, pl.ds(pr * 2 * GD, 2 * GD)],
                                               wq_v.at[pr, ks, :], sems.at[i]))
            for pr in REM.get(i, ()):
                kr = pl.ds(KM, D - KM)
                r.append(pltpu.make_async_copy(wq_hbm.at[kr, pl.ds(pr * 2 * GD, 2 * GD)],
                                               wq_v.at[pr, kr, :], sems.at[i]))
            return r

        pro_sets = [set_p(i) for i in range(NK)]

        def start(cps):
            for cp in cps:
                cp.start()

        def wait(cps):
            for cp in cps:
                cp.wait()

        for st in pro_sets:
            start(st)
        start(set_a())

        acc_ref[...] = jnp.zeros_like(acc_ref)

        def qp(pr, hf, qs, b):
            r0, r1 = b * Sq, (b + 1) * Sq
            if isinstance(pr, int) and pr in RSLOT:
                q = qacc_v[RSLOT[pr], r0:r1, half(hf)] + jnp.dot(
                    x_v[r0:r1, 0:KM], wq_v[pr, 0:KM, half(hf)], preferred_element_type=jnp.float32)
            else:
                q = jnp.dot(x_v[r0:r1, :], wq_v[pr, :, half(hf)],
                            preferred_element_type=jnp.float32)
            q_v[qs, r0:r1, :] = (q * scale).astype(jnp.bfloat16)

        def qk(u, qs, b, ps=0):
            for h in range(G):
                qb = q_v[qs, b * Sq:(b + 1) * Sq, h * Dh:(h + 1) * Dh]
                s = lax.dot_general(qb, k_v[b, u * G + h], _NT, preferred_element_type=jnp.float32)
                m = jnp.max(s, axis=-1, keepdims=True)
                p = jnp.exp(s - m)
                l = jnp.sum(p, axis=-1, keepdims=True)
                p_v[b % NPS, ps * G + h] = (p * pl.reciprocal(l, approx=True)).astype(jnp.bfloat16)

        def pv(u, slot, b, ps=0):
            for h in range(G):
                o = jnp.dot(p_v[b % NPS, ps * G + h], v_v[b, u * G + h],
                            preferred_element_type=jnp.float32)
                c0 = slot * GD + h * Dh
                a_v[b * Sq:(b + 1) * Sq, c0:c0 + Dh] = o.astype(jnp.bfloat16)

        def op(pr, slot, t):
            cs = slice(t * 128, (t + 1) * 128)
            at = a_v[cs, half(slot)]
            for r0 in range(0, D, OM):
                c = lax.dot_general(wo_v[pr, r0:r0 + OM, half(slot)], at, _NT,
                                    preferred_element_type=jnp.float32)
                acc_ref[r0:r0 + OM, cs] += c

        def op_nat(t, c0=0, c1=D):
            cs = slice(t * 128, (t + 1) * 128)
            tot = acct_v[NAT.index(t), :, c0:c1] + lax.dot_general(
                a_v[cs, :], wo_v[NP - 1, c0:c1, :], _NT, preferred_element_type=jnp.float32)
            o_v[cs, c0:c1] = tot.astype(o_v.dtype)

        def op2(pr, t):
            cs = slice(t * 128, (t + 1) * 128)
            if pr == NP - 1 and t in NAT:
                op_nat(t)
                return
            tot = acc_ref[:, cs] + lax.dot_general(wo_v[pr], a_v[cs, :], _NT,
                                                   preferred_element_type=jnp.float32)
            if pr == NP - 2 and t in NAT:
                acct_v[NAT.index(t)] = tot.T
            elif pr < NP - 1:
                acc_ref[:, cs] = tot
            else:
                o_v[cs, :] = tot.T.astype(o_v.dtype)

        def tail_pv(u, slot):
            pv(u, slot, B - 2)
            pv(u, slot, B - 1)

        OT = {0: 1, 1: 2, 3: 3, 4: 4, 5: 5}

        def unit_a(u):
            if u > 0:
                tail_pv(u - 1, u - 1)
            qk(u, u, 0)
            qk(u, u, 1)
            qp(2, u, u, 0)
            qk(u, u, 2)
            qp(2, u, u, 1)
            for b in range(B - 3):
                pv(u, u, b)
                qk(u, u, b + 3)
                qp(2, u, u, b + 2)
            pv(u, u, B - 3)
            qp(2, u, u, B - 1)

        def unit_b(pr, hf, qs):
            u = 2 * pr + hf
            tail_pv(u - 1, 1 - hf)
            qk(u, qs, 0)
            qk(u, qs, 1)
            op(pr - 1, hf, 0)
            qp(pr + 2, hf, qs, 0)
            for b in range(B - 2):
                pv(u, hf, b)
                qk(u, qs, b + 2)
                if b in OT:
                    op(pr - 1, hf, OT[b])
                qp(pr + 2, hf, qs, b + 1)
            qp(pr + 2, hf, qs, B - 1)

        def pair_b(pr):
            qb = (pr % 2) * 2
            unit_b(pr, 0, qb)
            unit_b(pr, 1, qb + 1)

        def qk2(pr, b):
            qb = (pr % 2) * 2
            qk(2 * pr, qb, b, 0)
            qk(2 * pr + 1, qb + 1, b, 1)

        def pv2(pr, b):
            pv(2 * pr, 0, b, 0)
            pv(2 * pr + 1, 1, b, 1)

        for i, st in enumerate(pro_sets):
            wait(st)
            k0, k1 = KSPLIT[i]
            if i < NK - 1:
                for r0 in range(0, M, PM):
                    for pr in range(2):
                        part = jnp.dot(x_v[r0:r0 + PM, k0:k1], wq_v[pr, k0:k1, :],
                                       preferred_element_type=jnp.float32)
                        if i > 0:
                            part = part + qacc_v[pr, r0:r0 + PM, :]
                        qacc_v[pr, r0:r0 + PM, :] = part
            else:
                for b in range(B):
                    r0, r1 = b * Sq, (b + 1) * Sq
                    for pr in range(2):
                        for hf in range(2):
                            q = qacc_v[pr, r0:r1, half(hf)] + jnp.dot(
                                x_v[r0:r1, k0:k1], wq_v[pr, k0:k1, half(hf)],
                                preferred_element_type=jnp.float32)
                            q_v[2 * pr + hf, r0:r1, :] = (q * scale).astype(jnp.bfloat16)
            for pr in REM.get(i, ()):
                for r0 in range(0, M, PM):
                    qacc_v[RSLOT[pr], r0:r0 + PM, :] = jnp.dot(
                        x_v[r0:r0 + PM, KM:D], wq_v[pr, KM:D, :],
                        preferred_element_type=jnp.float32)
            start(set_b(i + 1, i))
            if i == NK - 1:
                for pr in range(NK + 1, NB + 1):
                    start(set_b(pr, pr - 1))
                start(set_e())

        wait(set_a())
        unit_a(0)
        unit_a(1)

        def body_b(pr, carry):
            wait(set_b(pr, pr - 1))
            pair_b(pr)
            return carry

        lax.fori_loop(1, NB + 1, body_b, 0)

        wait(set_e())
        pair_b(NP - 3)
        c, e = NP - 2, NP - 1
        tail_pv(2 * c - 1, 1)
        qk2(c, 0); qk2(c, 1); op2(c - 1, 0)
        pv2(c, 0); qk2(c, 2); op2(c - 1, 1)
        pv2(c, 1); qk2(c, 3); op2(c - 1, 2)
        pv2(c, 2); qk2(c, 4); op2(c - 1, 3)
        pv2(c, 3); qk2(c, 5); op2(c - 1, 4)
        pv2(c, 4); qk2(c, 6); qk2(c, 7); op2(c - 1, 5)
        pv2(c, 5); qk2(e, 0); op2(c, 0)
        pv2(c, 6); pv2(c, 7); qk2(e, 1); op2(c, 1)
        pv2(e, 0); qk2(e, 2); op2(c, 2)
        pv2(e, 1); qk2(e, 3); op2(c, 3)
        pv2(e, 2); qk2(e, 4); op2(c, 4)
        pv2(e, 3); qk2(e, 5); op2(c, 5)
        pv2(e, 4); qk2(e, 6); op2(e, 0)
        cp_out(0).start()
        pv2(e, 5); qk2(e, 7); op2(e, 1)
        cp_out(1).start()
        op2(e, 2)
        cp_out(2).start()
        pv2(e, 6); op2(e, 3)
        cp_out(3).start()
        pv2(e, 7); op2(e, 4)
        cp_out(4).start()
        for (c0, c1) in CSPLIT:
            op_nat(NT - 1, c0, c1)
            cp_last(c0, c1).start()
        for t in range(NT - 1):
            cp_out(t).wait()
        for (c0, c1) in CSPLIT:
            cp_last(c0, c1).wait()

    out = pl.pallas_call(
        kernel,
        in_specs=[pl.BlockSpec(memory_space=pl.ANY)] * 5,
        out_specs=pl.BlockSpec(memory_space=pl.ANY),
        out_shape=jax.ShapeDtypeStruct((M, D), x.dtype),
        scratch_shapes=[
            pltpu.VMEM((M, D), jnp.bfloat16),
            pltpu.VMEM((NP, D, 2 * GD), jnp.bfloat16),
            pltpu.VMEM((B, H, Sk, Dh), jnp.bfloat16),
            pltpu.VMEM((B, H, Sk, Dh), jnp.bfloat16),
            pltpu.VMEM((NP, D, 2 * GD), jnp.bfloat16),
            pltpu.VMEM((D, M), jnp.float32),
            pltpu.VMEM((4, M, GD), jnp.bfloat16),
            pltpu.VMEM((NPS, 2 * G, Sq, Sk), jnp.bfloat16),
            pltpu.VMEM((M, 2 * GD), jnp.bfloat16),
            pltpu.VMEM((M, D), jnp.bfloat16),
            pltpu.VMEM((len(NAT), 128, D), jnp.float32),
            pltpu.VMEM((2 + len(RSLOT), M, 2 * GD), jnp.float32),
            pltpu.SemaphoreType.DMA((NSEM,)),
        ],
        compiler_params=pltpu.CompilerParams(
            vmem_limit_bytes=100 * 1024 * 1024,
        ),
    )(x2, wq, k_cache, v_cache, woT)
    return out.reshape(B, Sq, D)
```
